```python
import os as _os
_os.environ.setdefault("JAX_PLATFORMS", "cpu")
import jax
import jax.numpy as jnp

def _softmax(x, axis=-1):
    return jax.nn.softmax(x, axis=axis)
def _gelu(x):
    return jax.nn.gelu(x, approximate=True)
def _silu(x):
    return jax.nn.silu(x)
def _sigmoid(x):
    return jax.nn.sigmoid(x)
def _layernorm(x, axis=-1, eps=1e-5):
    m = jnp.mean(x, axis=axis, keepdims=True)
    v = jnp.var(x, axis=axis, keepdims=True)
    return (x - m) / jnp.sqrt(v + eps)
def _scatter_add(tgt, idx, src, axis=0):
    return tgt.at[idx].add(src)
def _segment_sum(src, seg, n):
    return jax.ops.segment_sum(src, seg, n)
class _Rng:
    def __init__(self, key):
        self._k = key
    def _next(self):
        self._k, sub = jax.random.split(self._k)
        return sub
    def normal(self, shape):
        return jax.random.normal(self._next(), shape, dtype=jnp.bfloat16)
    def randint(self, lo, hi, shape):
        return jax.random.randint(self._next(), shape, lo, hi, dtype=jnp.int32)
    def uniform(self, shape, lo=0.0, hi=1.0):
        return jax.random.uniform(self._next(), shape, jnp.bfloat16, lo, hi)
    def permutation(self, n):
        return jax.random.permutation(self._next(), n)


kernel_name = 'standalone__instancenorm__sampling'

def setup_inputs():
    _rng = _Rng(jax.random.key(int.from_bytes(__import__("os").urandom(4), "little")))
    _w = (lambda a: (lambda t: t.astype(jnp.bfloat16) if jnp.issubdtype(t.dtype, jnp.floating) else t)(jnp.asarray(a)))
    B, C, H, W = 16, 640, 16, 32
    return {
        "x": _w((lambda *s: _rng.normal(s) * 0.05)(B, C, H, W)),
        "g": _w((lambda *s: _rng.normal(s) * 0.05)(C) + 1.0),
        "b": _w((lambda *s: _rng.normal(s) * 0.05)(C)),
    }

def reference(x, g, b):
    mu = x.mean(axis=(-2, -1), keepdims=True)
    var = ((x - mu) * (x - mu)).mean(axis=(-2, -1), keepdims=True)
    xhat = (x - mu) / jnp.sqrt(var + 1e-5)
    return xhat * g.reshape(1, -1, 1, 1) + b.reshape(1, -1, 1, 1)
```

```python
import jax
import jax.numpy as jnp
import jax.experimental.pallas as pl
import jax.experimental.pallas.tpu as pltpu

_EPS = 1e-5
_NB = 1
_WIN = 2
_EARLY = 1


@jax.jit
def pallas_standalone__instancenorm__sampling_kernel(
    x: jax.Array,
    g: jax.Array,
    b: jax.Array,
):
    B, C, H, W = x.shape
    HW = H * W
    nb = _NB
    N = B // nb
    win = _WIN
    xt = jnp.transpose(x, (0, 2, 3, 1)).reshape(B, HW, C)

    def kernel(x_hbm, g_hbm, b_hbm, o_hbm, buf, gbuf, bbuf, rsem, wsem, psem):
        def rd(k):
            return pltpu.make_async_copy(
                x_hbm.at[pl.ds(k * nb, nb)], buf.at[pl.ds(k * nb, nb)], rsem.at[k])

        def wr(k, n=1):
            return pltpu.make_async_copy(
                buf.at[pl.ds(k * nb, n * nb)], o_hbm.at[pl.ds(k * nb, n * nb)], wsem.at[k])

        gc = pltpu.make_async_copy(g_hbm, gbuf, psem.at[0])
        bc = pltpu.make_async_copy(b_hbm, bbuf, psem.at[1])
        gc.start()
        bc.start()
        for k in range(min(win, N)):
            rd(k).start()
        gc.wait()
        bc.wait()
        gg = gbuf[...].astype(jnp.float32).reshape(1, C)
        bv = bbuf[...].astype(jnp.float32).reshape(1, C)

        def compute(k):
            for i in range(nb):
                idx = k * nb + i
                xv = buf[idx].astype(jnp.float32)
                mu = jnp.sum(xv, axis=0, keepdims=True) * (1.0 / HW)
                xc = xv - mu
                var = jnp.sum(xc * xc, axis=0, keepdims=True) * (1.0 / HW)
                scale = gg * jax.lax.rsqrt(var + _EPS)
                buf[idx] = (xc * scale + bv).astype(buf.dtype)

        K = N - 1 - _EARLY

        def body(k, c):
            rd(k).wait()

            @pl.when(k + win < N)
            def _():
                rd(k + win).start()

            compute(k)
            return c

        jax.lax.fori_loop(0, K, body, 0)
        rd(K).wait()
        if K + win < N:
            rd(K + win).start()
        wr(0, K).start()
        for k in range(K, N):
            if k > K:
                rd(k).wait()
                if k + win < N:
                    rd(k + win).start()
            compute(k)
            wr(k).start()
        wr(0, K).wait()
        for k in range(K, N):
            wr(k).wait()

    out = pl.pallas_call(
        kernel,
        in_specs=[pl.BlockSpec(memory_space=pl.ANY)] * 3,
        out_specs=pl.BlockSpec(memory_space=pl.ANY),
        out_shape=jax.ShapeDtypeStruct((B, HW, C), x.dtype),
        scratch_shapes=[
            pltpu.VMEM((B, HW, C), x.dtype),
            pltpu.VMEM((C,), g.dtype),
            pltpu.VMEM((C,), b.dtype),
            pltpu.SemaphoreType.DMA((N,)),
            pltpu.SemaphoreType.DMA((N,)),
            pltpu.SemaphoreType.DMA((2,)),
        ],
        compiler_params=pltpu.CompilerParams(vmem_limit_bytes=64 * 1024 * 1024),
    )(xt, g, b)
    return jnp.transpose(out.reshape(B, H, W, C), (0, 3, 1, 2))
```

```python
import jax
import jax.numpy as jnp
import jax.experimental.pallas as pl
import jax.experimental.pallas.tpu as pltpu

_EPS = 1e-5


@jax.jit
def pallas_standalone__instancenorm__sampling_kernel(
    x: jax.Array,
    g: jax.Array,
    b: jax.Array,
):
    B, C, H, W = x.shape
    HW = H * W
    R = B * HW
    a = B // 2
    tail = HW // 2
    assert B >= 2 and tail % 16 == 0 and HW % 16 == 0
    rows = (a * HW, R - a * HW - tail, tail)
    offs = (0, rows[0], rows[0] + rows[1])

    xt = jnp.transpose(x, (0, 2, 3, 1)).reshape(R, C)

    def kernel(x_hbm, g_hbm, b_hbm, o_hbm, buf, gbuf, bbuf, rsem, wsem, psem):
        def rd(j):
            sl = pl.ds(offs[j], rows[j])
            return pltpu.make_async_copy(x_hbm.at[sl], buf.at[sl], rsem.at[j])

        def wr(j, b0, b1):
            sl = pl.ds(b0 * HW, (b1 - b0) * HW)
            return pltpu.make_async_copy(buf.at[sl], o_hbm.at[sl], wsem.at[j])

        g_cp = pltpu.make_async_copy(g_hbm, gbuf, psem.at[0])
        b_cp = pltpu.make_async_copy(b_hbm, bbuf, psem.at[1])
        g_cp.start()
        b_cp.start()
        rd(0).start()
        g_cp.wait()
        b_cp.wait()
        rd(1).start()
        rd(2).start()
        gamma = gbuf[...].astype(jnp.float32).reshape(1, C)
        beta = bbuf[...].astype(jnp.float32).reshape(1, C)

        def normalize(bi, carry):
            sl = pl.ds(pl.multiple_of(bi * HW, HW), HW)
            xv = buf[sl, :].astype(jnp.float32)
            mu = jnp.sum(xv, axis=0, keepdims=True) * (1.0 / HW)
            xc = xv - mu
            var = jnp.sum(xc * xc, axis=0, keepdims=True) * (1.0 / HW)
            scale = gamma * jax.lax.rsqrt(var + _EPS)
            buf[sl, :] = (xc * scale + beta).astype(buf.dtype)
            return carry

        rd(0).wait()
        jax.lax.fori_loop(0, a, normalize, 0)
        rd(1).wait()
        wr(0, 0, a).start()
        rd(2).wait()
        jax.lax.fori_loop(a, B, normalize, 0)
        wr(1, a, B).start()
        wr(0, 0, a).wait()
        wr(1, a, B).wait()

    out = pl.pallas_call(
        kernel,
        in_specs=[pl.BlockSpec(memory_space=pl.ANY)] * 3,
        out_specs=pl.BlockSpec(memory_space=pl.ANY),
        out_shape=jax.ShapeDtypeStruct((R, C), x.dtype),
        scratch_shapes=[
            pltpu.VMEM((R, C), x.dtype),
            pltpu.VMEM((C,), g.dtype),
            pltpu.VMEM((C,), b.dtype),
            pltpu.SemaphoreType.DMA((3,)),
            pltpu.SemaphoreType.DMA((2,)),
            pltpu.SemaphoreType.DMA((2,)),
        ],
        compiler_params=pltpu.CompilerParams(vmem_limit_bytes=48 * 1024 * 1024),
    )(xt, g, b)
    return jnp.transpose(out.reshape(B, H, W, C), (0, 3, 1, 2))
```
